```python
import os as _os
_os.environ.setdefault("JAX_PLATFORMS", "cpu")
import jax
import jax.numpy as jnp

def _softmax(x, axis=-1):
    return jax.nn.softmax(x, axis=axis)
def _gelu(x):
    return jax.nn.gelu(x, approximate=True)
def _silu(x):
    return jax.nn.silu(x)
def _sigmoid(x):
    return jax.nn.sigmoid(x)
def _layernorm(x, axis=-1, eps=1e-5):
    m = jnp.mean(x, axis=axis, keepdims=True)
    v = jnp.var(x, axis=axis, keepdims=True)
    return (x - m) / jnp.sqrt(v + eps)
def _scatter_add(tgt, idx, src, axis=0):
    return tgt.at[idx].add(src)
def _segment_sum(src, seg, n):
    return jax.ops.segment_sum(src, seg, n)
class _Rng:
    def __init__(self, key):
        self._k = key
    def _next(self):
        self._k, sub = jax.random.split(self._k)
        return sub
    def normal(self, shape):
        return jax.random.normal(self._next(), shape, dtype=jnp.bfloat16)
    def randint(self, lo, hi, shape):
        return jax.random.randint(self._next(), shape, lo, hi, dtype=jnp.int32)
    def uniform(self, shape, lo=0.0, hi=1.0):
        return jax.random.uniform(self._next(), shape, jnp.bfloat16, lo, hi)
    def permutation(self, n):
        return jax.random.permutation(self._next(), n)


kernel_name = 'sequential_preLN__compressed_kv_cla__dense_activation_mish__decode'

def setup_inputs():
    _rng = _Rng(jax.random.key(int.from_bytes(__import__("os").urandom(4), "little")))
    _w = (lambda a: (lambda t: t.astype(jnp.bfloat16) if jnp.issubdtype(t.dtype, jnp.floating) else t)(jnp.asarray(a)))
    def _A_setup():
        B, H, Sq, Sk, D, M = 2, 32, 1, 8192, 128, 512
        Dc = 4 * D
        return {
            "x": _w((lambda *s: _rng.normal(s) * 0.05)(B, Sq, M)),
            "c_kv": _w((lambda *s: _rng.normal(s) * 0.8)(B, Sk, Dc)),
            "w_q": _w((lambda *s: _rng.normal(s) * 0.8)(M, H, D) * (M ** -0.5)),
            "w_uk": _w((lambda *s: _rng.normal(s) * 0.8)(Dc, H, D) * (Dc ** -0.5)),
            "w_uv": _w((lambda *s: _rng.normal(s) * 0.8)(Dc, H, D) * (Dc ** -0.5)),
            "w_o": _w((lambda *s: _rng.normal(s) * 0.8)(H, D, M) * ((H * D) ** -0.5)),
        }
    _A_in = _A_setup()

    def _B_setup():
        B, S, D, F = 2, 1, 512, 1792
        return {
            "x": _w((lambda *s: _rng.normal(s) * 0.05)(B, S, D)),
            "w1": _w((lambda *s: _rng.normal(s) * 0.4)(D, F) * (D ** -0.5)),
            "b1": _w((lambda *s: _rng.normal(s) * 0.05)(F)),
            "w2": _w((lambda *s: _rng.normal(s) * 0.05)(F, D) * (F ** -0.5)),
        }
    _B_in = _B_setup()

    return {
        "A_x": _A_in["x"],
        "A_c_kv": _A_in["c_kv"],
        "A_w_q": _A_in["w_q"],
        "A_w_uk": _A_in["w_uk"],
        "A_w_uv": _A_in["w_uv"],
        "A_w_o": _A_in["w_o"],
        "B_x": _B_in["x"],
        "B_w1": _B_in["w1"],
        "B_b1": _B_in["b1"],
        "B_w2": _B_in["w2"],
    }

def reference(A_x, A_c_kv, A_w_q, A_w_uk, A_w_uv, A_w_o, B_x, B_w1, B_b1, B_w2):
    def _A_ref(x, c_kv, w_q, w_uk, w_uv, w_o):
        B, Sq, M = x.shape[0], x.shape[1], x.shape[2]
        Sk = c_kv.shape[1]
        H, D = w_q.shape[1], w_q.shape[2]
        q = jnp.einsum("bqm,mhd->bhqd", x, w_q)
        k = jnp.einsum("bkc,chd->bhkd", c_kv, w_uk)
        v = jnp.einsum("bkc,chd->bhkd", c_kv, w_uv)
        scores = jnp.einsum("bhqd,bhkd->bhqk", q, k) * (D ** -0.5)
        off = Sk - Sq
        qi = jnp.arange(Sq)[:, None]
        kj = jnp.arange(Sk)[None, :]
        cmask = kj <= (qi + off)
        scores = jnp.where(cmask[None, None], scores, -1e9)
        p = _softmax(scores, axis=-1)
        ctx = jnp.einsum("bhqk,bhkd->bhqd", p, v)
        return jnp.einsum("bhqd,hdm->bqm", ctx, w_o)

    def _B_ref(x, w1, b1, w2):
        h = jnp.einsum("bsd,df->bsf", x, w1) + b1
        sp = jnp.log1p(jnp.exp(-jnp.abs(h))) + jnp.where(h > 0, h, jnp.zeros_like(h))
        act = h * jnp.tanh(sp)
        return jnp.einsum("bsf,fd->bsd", act, w2)

    x = A_x
    h = x + _A_ref(_layernorm(x, axis=-1), A_c_kv, A_w_q, A_w_uk, A_w_uv, A_w_o)
    h2 = h + _B_ref(_layernorm(h, axis=-1), B_w1, B_b1, B_w2)
    return h2
```

```python
import functools

import jax
import jax.numpy as jnp
import jax.experimental.pallas as pl
import jax.experimental.pallas.tpu as pltpu

_B, _H, _SK, _D, _M = 2, 32, 8192, 128, 512
_DC = 4 * _D
_F = 1792
_EPS = 1e-5

_TK = 1024
_NCK = _B * _SK // _TK
_CPB = _SK // _TK
_NWC = 4
_W1C = 4
_W2C = 7

_S_X = 0
_S_WQ = _S_X + 1
_S_WUK = _S_WQ + _NWC
_S_CKV = _S_WUK + _NWC
_S_WUV = _S_CKV + _NCK
_S_WO = _S_WUV + _NWC
_S_B1 = _S_WO + _NWC
_S_W1 = _S_B1 + 1
_S_W2 = _S_W1 + _W1C
_NSEM = _S_W2 + _W2C


def _rows16(v2):
    n = v2.shape[1]
    return jnp.concatenate(
        [jnp.broadcast_to(v2[0:1, :], (8, n)), jnp.broadcast_to(v2[1:2, :], (8, n))], axis=0)


def _layernorm(v):
    m = jnp.mean(v, axis=-1, keepdims=True)
    c = v - m
    var = jnp.mean(c * c, axis=-1, keepdims=True)
    return c * jax.lax.rsqrt(var + _EPS)


def _kernel(x_hbm, ckv_hbm, wq_hbm, wuk_hbm, wuv_hbm, wo_hbm, w1_hbm, b1_hbm, w2_hbm,
            out_ref,
            x_v, ckv_v, wq_v, wuk_v, wuv_v, wo_v, w1_v, b1_v, w2_v,
            e2_v, qabs_f, qabs_b, m_s, l_s, acc_s, sems):
    f32, bf16 = jnp.float32, jnp.bfloat16

    def cp_x():
        return pltpu.make_async_copy(x_hbm, x_v, sems.at[_S_X])

    def cp_w3(hbm, vmem, sbase, g):
        return pltpu.make_async_copy(hbm.at[pl.ds(4096 * g, 4096)], vmem.at[pl.ds(4096 * g, 4096)],
                                     sems.at[sbase + g])

    def cp_ckv(i):
        return pltpu.make_async_copy(ckv_hbm.at[pl.ds(_TK * i, _TK)], ckv_v.at[pl.ds(_TK * i, _TK)],
                                     sems.at[_S_CKV + i])

    def cp_wo(g):
        return pltpu.make_async_copy(wo_hbm.at[pl.ds(1024 * g, 1024)], wo_v.at[pl.ds(1024 * g, 1024)],
                                     sems.at[_S_WO + g])

    def cp_b1():
        return pltpu.make_async_copy(b1_hbm, b1_v, sems.at[_S_B1])

    def cp_w1(g):
        return pltpu.make_async_copy(w1_hbm.at[pl.ds(128 * g, 128)], w1_v.at[pl.ds(128 * g, 128)],
                                     sems.at[_S_W1 + g])

    def cp_w2(g):
        return pltpu.make_async_copy(w2_hbm.at[pl.ds(256 * g, 256)], w2_v.at[pl.ds(256 * g, 256)],
                                     sems.at[_S_W2 + g])

    cp_x().start()
    for g in range(_NWC):
        cp_w3(wq_hbm, wq_v, _S_WQ, g).start()
    for g in range(_NWC):
        cp_w3(wuk_hbm, wuk_v, _S_WUK, g).start()
    for i in range(_NCK):
        cp_ckv(i).start()
    for g in range(_NWC):
        cp_w3(wuv_hbm, wuv_v, _S_WUV, g).start()
    for g in range(_NWC):
        cp_wo(g).start()
    cp_b1().start()
    for g in range(_W1C):
        cp_w1(g).start()
    for g in range(_W2C):
        cp_w2(g).start()

    ri = jax.lax.broadcasted_iota(jnp.int32, (128, 1024), 0)
    li = jax.lax.broadcasted_iota(jnp.int32, (128, 1024), 1)
    e2_v[...] = jnp.where((li % 256) // 2 == ri, 1.0, 0.0).astype(bf16)

    def pairmask():
        r = jax.lax.broadcasted_iota(jnp.int32, (16, 1024), 0) % 8
        l = jax.lax.broadcasted_iota(jnp.int32, (16, 1024), 1)
        return jnp.logical_and(l // 256 == r // 2, l % 2 == r % 2)

    def rhscat(w_v, g, i):
        w32 = w_v.bitcast(jnp.uint32)
        parts = [w32[pl.ds(2048 * g + 4 * i + t, 128, stride=16), :] for t in range(4)]
        return pltpu.bitcast(jnp.concatenate(parts, axis=0), bf16)

    cp_x().wait()
    x2 = x_v[...].astype(f32)
    lnx16 = _rows16(_layernorm(x2)).astype(bf16)

    pm = pairmask()
    qg = [jnp.zeros((16, _D), f32) for _ in range(4)]
    for g in range(_NWC):
        lhs = jnp.dot(lnx16[:, 128 * g:128 * (g + 1)], e2_v[...], preferred_element_type=f32)
        lhs = jnp.where(pm, lhs, 0.0).astype(bf16)
        cp_w3(wq_hbm, wq_v, _S_WQ, g).wait()
        for i in range(4):
            qg[i] = qg[i] + jnp.dot(lhs, rhscat(wq_v, g, i), preferred_element_type=f32)
    qb = [q.astype(bf16) for q in qg]

    scale = float(_D) ** -0.5
    for g in range(_NWC):
        cp_w3(wuk_hbm, wuk_v, _S_WUK, g).wait()
        ex = []
        for i in range(4):
            o = jax.lax.dot_general(qb[i], rhscat(wuk_v, g, i), (((1,), (1,)), ((), ())),
                                    preferred_element_type=f32)
            ex.append(jnp.where(pm, o * scale, 0.0).astype(bf16))
        exc = jnp.concatenate(ex, axis=0)
        qa = jax.lax.dot_general(exc, e2_v[...], (((1,), (1,)), ((), ())),
                                 preferred_element_type=f32)
        for i in range(4):
            for b in range(_B):
                qabs_f[pl.ds(32 * b + 8 * i, 8), pl.ds(128 * g, 128)] = qa[16 * i + 8 * b:16 * i + 8 * b + 8, :]
    qabs_b[...] = qabs_f[...].astype(bf16)

    m_s[...] = jnp.full(m_s.shape, -jnp.inf, f32)
    l_s[...] = jnp.zeros(l_s.shape, f32)
    acc_s[...] = jnp.zeros(acc_s.shape, f32)

    def ck_body(i, carry):
        b = i // _CPB
        cp_ckv(i).wait()
        ck = ckv_v[pl.ds(pl.multiple_of(i * _TK, _TK), _TK), :]
        qa = qabs_b[pl.ds(pl.multiple_of(32 * b, 32), 32), :]
        s = jax.lax.dot_general(qa, ck, (((1,), (1,)), ((), ())), preferred_element_type=f32)
        m_prev = m_s[b]
        m_new = jnp.maximum(m_prev, jnp.max(s, axis=1, keepdims=True))
        p = jnp.exp(s - m_new)
        alpha = jnp.exp(m_prev - m_new)
        l_s[b] = alpha * l_s[b] + jnp.sum(p, axis=1, keepdims=True)
        acc_s[b] = alpha * acc_s[b] + jnp.dot(p.astype(bf16), ck, preferred_element_type=f32)
        m_s[b] = m_new
        return carry

    jax.lax.fori_loop(0, _NCK, ck_body, 0)

    ctxc = jnp.concatenate([acc_s[0] / l_s[0], acc_s[1] / l_s[1]], axis=0).astype(bf16)

    pm = pairmask()
    cg = [jnp.zeros((16, _D), f32) for _ in range(4)]
    for g in range(_NWC):
        zx = jnp.dot(ctxc[:, 128 * g:128 * (g + 1)], e2_v[...], preferred_element_type=f32)
        cp_w3(wuv_hbm, wuv_v, _S_WUV, g).wait()
        for i in range(4):
            z16 = jnp.concatenate([zx[8 * i:8 * i + 8, :], zx[32 + 8 * i:32 + 8 * i + 8, :]], axis=0)
            lhs = jnp.where(pm, z16, 0.0).astype(bf16)
            cg[i] = cg[i] + jnp.dot(lhs, rhscat(wuv_v, g, i), preferred_element_type=f32)

    hr = jax.lax.broadcasted_iota(jnp.int32, (16, 1024), 0) % 8
    hl = jax.lax.broadcasted_iota(jnp.int32, (16, 1024), 1) // 128
    hmask = hr == hl
    ao = jnp.zeros((16, _M), f32)
    for g in range(_NWC):
        ct = jnp.concatenate([cg[g]] * 8, axis=1)
        lhs = jnp.where(hmask, ct, 0.0).astype(bf16)
        cp_wo(g).wait()
        ao = ao + jnp.dot(lhs, wo_v[pl.ds(1024 * g, 1024), :], preferred_element_type=f32)
    attn = jnp.concatenate([jnp.sum(ao[0:8, :], axis=0, keepdims=True),
                            jnp.sum(ao[8:16, :], axis=0, keepdims=True)], axis=0)
    h = x2 + attn

    lnh16 = _rows16(_layernorm(h)).astype(bf16)
    cp_b1().wait()
    h1 = jnp.broadcast_to(b1_v[...].astype(f32).reshape(1, _F), (16, _F))
    for g in range(_W1C):
        cp_w1(g).wait()
        h1 = h1 + jnp.dot(lnh16[:, 128 * g:128 * (g + 1)], w1_v[pl.ds(128 * g, 128), :],
                          preferred_element_type=f32)
    sp = jnp.log1p(jnp.exp(-jnp.abs(h1))) + jnp.maximum(h1, 0.0)
    act = (h1 * jnp.tanh(sp)).astype(bf16)
    y = jnp.zeros((16, _M), f32)
    for g in range(_W2C):
        cp_w2(g).wait()
        y = y + jnp.dot(act[:, 256 * g:256 * (g + 1)], w2_v[pl.ds(256 * g, 256), :],
                        preferred_element_type=f32)
    out_ref[...] = (h + jnp.concatenate([y[0:1, :], y[8:9, :]], axis=0)).astype(out_ref.dtype)


@jax.jit
def pallas_sequential_preLN__compressed_kv_cla__dense_activation_mish__decode_kernel(
    A_x: jax.Array,
    A_c_kv: jax.Array,
    A_w_q: jax.Array,
    A_w_uk: jax.Array,
    A_w_uv: jax.Array,
    A_w_o: jax.Array,
    B_x: jax.Array,
    B_w1: jax.Array,
    B_b1: jax.Array,
    B_w2: jax.Array,
):
    del B_x
    bf16 = jnp.bfloat16
    x2d = A_x.reshape(_B, _M)
    ckv2 = A_c_kv.reshape(_B * _SK, _DC)
    wq2 = A_w_q.reshape(_M * _H, _D)
    wuk2 = A_w_uk.reshape(_DC * _H, _D)
    wuv2 = A_w_uv.reshape(_DC * _H, _D)
    wo2 = A_w_o.reshape(_H * _D, _M)

    any_spec = pl.BlockSpec(memory_space=pl.ANY)
    out = pl.pallas_call(
        _kernel,
        out_shape=jax.ShapeDtypeStruct((_B, _M), A_x.dtype),
        in_specs=[any_spec] * 9,
        out_specs=pl.BlockSpec(memory_space=pltpu.VMEM),
        scratch_shapes=[
            pltpu.VMEM((_B, _M), bf16),
            pltpu.VMEM((_B * _SK, _DC), bf16),
            pltpu.VMEM((_M * _H, _D), bf16),
            pltpu.VMEM((_DC * _H, _D), bf16),
            pltpu.VMEM((_DC * _H, _D), bf16),
            pltpu.VMEM((_H * _D, _M), bf16),
            pltpu.VMEM((_M, _F), bf16),
            pltpu.VMEM((_F,), bf16),
            pltpu.VMEM((_F, _M), bf16),
            pltpu.VMEM((128, 1024), bf16),
            pltpu.VMEM((_B * _H, _DC), jnp.float32),
            pltpu.VMEM((_B * _H, _DC), bf16),
            pltpu.VMEM((_B, _H, 1), jnp.float32),
            pltpu.VMEM((_B, _H, 1), jnp.float32),
            pltpu.VMEM((_B, _H, _DC), jnp.float32),
            pltpu.SemaphoreType.DMA((_NSEM,)),
        ],
        compiler_params=pltpu.CompilerParams(vmem_limit_bytes=64 * 1024 * 1024),
    )(x2d, ckv2, wq2, wuk2, wuv2, wo2, B_w1, B_b1, B_w2)
    return out.reshape(_B, 1, _M)
```

```python
import jax
import jax.numpy as jnp
import jax.experimental.pallas as pl
import jax.experimental.pallas.tpu as pltpu

_B, _H, _SK, _D, _M = 2, 32, 8192, 128, 512
_DC = 4 * _D
_F = 1792
_EPS = 1e-5

_TK = 1024
_DK = 2048
_NDK = _B * _SK // _DK
_DPB = _SK // _DK
_NWC = 4
_W2_PIECES = ((0, 1280), (1280, 256), (1536, 256))

_S_X = 0
_S_WQ = 1
_S_WUK = 2
_S_CKV = 3
_S_WUV = _S_CKV + _NDK
_S_WO = _S_WUV + 1
_S_B1 = _S_WO + 1
_S_W1 = _S_B1 + 1
_S_W2 = _S_W1 + 1
_NSEM = _S_W2 + len(_W2_PIECES)


def _rows16(v2):
    n = v2.shape[1]
    return jnp.concatenate(
        [jnp.broadcast_to(v2[0:1, :], (8, n)), jnp.broadcast_to(v2[1:2, :], (8, n))], axis=0)


def _layernorm(v):
    m = jnp.mean(v, axis=-1, keepdims=True)
    c = v - m
    var = jnp.mean(c * c, axis=-1, keepdims=True)
    return c * jax.lax.rsqrt(var + _EPS)


def _kernel(x_hbm, ckv_hbm, wq_hbm, wuk_hbm, wuv_hbm, wo_hbm, w1_hbm, b1_hbm, w2_hbm,
            out_ref,
            x_v, ckv_v, wq_v, wuk_v, wuv_v, wo_v, w1_v, b1_v, w2_v,
            e2_v, qabs_f, qabs_b, m_s, l_s, acc_s, sems):
    f32, bf16 = jnp.float32, jnp.bfloat16

    def cp_x():
        return pltpu.make_async_copy(x_hbm, x_v, sems.at[_S_X])

    def cp_ckv(i):
        return pltpu.make_async_copy(ckv_hbm.at[pl.ds(_DK * i, _DK)], ckv_v.at[pl.ds(_DK * i, _DK)],
                                     sems.at[_S_CKV + i])

    def cp_w2(k):
        off, n = _W2_PIECES[k]
        return pltpu.make_async_copy(w2_hbm.at[pl.ds(off, n)], w2_v.at[pl.ds(off, n)],
                                     sems.at[_S_W2 + k])

    cp_wq = pltpu.make_async_copy(wq_hbm, wq_v, sems.at[_S_WQ])
    cp_wuk = pltpu.make_async_copy(wuk_hbm, wuk_v, sems.at[_S_WUK])
    cp_wuv = pltpu.make_async_copy(wuv_hbm, wuv_v, sems.at[_S_WUV])
    cp_wo = pltpu.make_async_copy(wo_hbm, wo_v, sems.at[_S_WO])
    cp_b1 = pltpu.make_async_copy(b1_hbm, b1_v, sems.at[_S_B1])
    cp_w1 = pltpu.make_async_copy(w1_hbm, w1_v, sems.at[_S_W1])

    cp_x().start()
    cp_wq.start()
    cp_wuk.start()
    for i in range(_NDK):
        cp_ckv(i).start()
    cp_wuv.start()
    cp_wo.start()
    cp_b1.start()
    cp_w1.start()
    for k in range(len(_W2_PIECES)):
        cp_w2(k).start()

    ri = jax.lax.broadcasted_iota(jnp.int32, (128, 1024), 0)
    li = jax.lax.broadcasted_iota(jnp.int32, (128, 1024), 1)
    e2_v[...] = jnp.where((li % 256) // 2 == ri, 1.0, 0.0).astype(bf16)

    def pairmask():
        r = jax.lax.broadcasted_iota(jnp.int32, (16, 1024), 0) % 8
        l = jax.lax.broadcasted_iota(jnp.int32, (16, 1024), 1)
        return jnp.logical_and(l // 256 == r // 2, l % 2 == r % 2)

    def rhscat(w_v, g, i):
        w32 = w_v.bitcast(jnp.uint32)
        parts = [w32[pl.ds(2048 * g + 4 * i + t, 128, stride=16), :] for t in range(4)]
        return pltpu.bitcast(jnp.concatenate(parts, axis=0), bf16)

    cp_x().wait()
    x2 = x_v[...].astype(f32)
    lnx16 = _rows16(_layernorm(x2)).astype(bf16)

    pm = pairmask()
    qg = [jnp.zeros((16, _D), f32) for _ in range(4)]
    for g in range(_NWC):
        lhs = jnp.dot(lnx16[:, 128 * g:128 * (g + 1)], e2_v[...], preferred_element_type=f32)
        lhs = jnp.where(pm, lhs, 0.0).astype(bf16)
        if g == 0:
            cp_wq.wait()
        for i in range(4):
            qg[i] = qg[i] + jnp.dot(lhs, rhscat(wq_v, g, i), preferred_element_type=f32)
    qb = [q.astype(bf16) for q in qg]

    scale = float(_D) ** -0.5
    cp_wuk.wait()
    for g in range(_NWC):
        ex = []
        for i in range(4):
            o = jax.lax.dot_general(qb[i], rhscat(wuk_v, g, i), (((1,), (1,)), ((), ())),
                                    preferred_element_type=f32)
            ex.append(jnp.where(pm, o * scale, 0.0).astype(bf16))
        exc = jnp.concatenate(ex, axis=0)
        qa = jax.lax.dot_general(exc, e2_v[...], (((1,), (1,)), ((), ())),
                                 preferred_element_type=f32)
        for i in range(4):
            for b in range(_B):
                qabs_f[pl.ds(32 * b + 8 * i, 8), pl.ds(128 * g, 128)] = qa[16 * i + 8 * b:16 * i + 8 * b + 8, :]
    qabs_b[...] = qabs_f[...].astype(bf16)

    m_s[...] = jnp.full(m_s.shape, -jnp.inf, f32)
    l_s[...] = jnp.zeros(l_s.shape, f32)
    acc_s[...] = jnp.zeros(acc_s.shape, f32)

    def ck_body(i, carry):
        b = i // _DPB
        cp_ckv(i).wait()
        qa = qabs_b[pl.ds(pl.multiple_of(32 * b, 32), 32), :]
        for u in range(_DK // _TK):
            start = pl.multiple_of(i * _DK + u * _TK, _TK)
            ck = ckv_v[pl.ds(start, _TK), :]
            s = jax.lax.dot_general(qa, ck, (((1,), (1,)), ((), ())), preferred_element_type=f32)
            m_prev = m_s[b]
            m_new = jnp.maximum(m_prev, jnp.max(s, axis=1, keepdims=True))
            p = jnp.exp(s - m_new)
            alpha = jnp.exp(m_prev - m_new)
            l_s[b] = alpha * l_s[b] + jnp.sum(p, axis=1, keepdims=True)
            acc_s[b] = alpha * acc_s[b] + jnp.dot(p.astype(bf16), ck, preferred_element_type=f32)
            m_s[b] = m_new
        return carry

    jax.lax.fori_loop(0, _NDK, ck_body, 0)

    ctxc = jnp.concatenate([acc_s[0] / l_s[0], acc_s[1] / l_s[1]], axis=0).astype(bf16)

    pm = pairmask()
    cg = [jnp.zeros((16, _D), f32) for _ in range(4)]
    for g in range(_NWC):
        zx = jnp.dot(ctxc[:, 128 * g:128 * (g + 1)], e2_v[...], preferred_element_type=f32)
        if g == 0:
            cp_wuv.wait()
        for i in range(4):
            z16 = jnp.concatenate([zx[8 * i:8 * i + 8, :], zx[32 + 8 * i:32 + 8 * i + 8, :]], axis=0)
            lhs = jnp.where(pm, z16, 0.0).astype(bf16)
            cg[i] = cg[i] + jnp.dot(lhs, rhscat(wuv_v, g, i), preferred_element_type=f32)

    hr = jax.lax.broadcasted_iota(jnp.int32, (16, 1024), 0) % 8
    hl = jax.lax.broadcasted_iota(jnp.int32, (16, 1024), 1) // 128
    hmask = hr == hl
    lhs_o = jnp.concatenate(
        [jnp.where(hmask, jnp.concatenate([cg[g]] * 8, axis=1), 0.0).astype(bf16) for g in range(4)],
        axis=1)
    cp_wo.wait()
    ao = jnp.dot(lhs_o, wo_v[...], preferred_element_type=f32)
    attn = jnp.concatenate([jnp.sum(ao[0:8, :], axis=0, keepdims=True),
                            jnp.sum(ao[8:16, :], axis=0, keepdims=True)], axis=0)
    h = x2 + attn

    lnh16 = _rows16(_layernorm(h)).astype(bf16)
    cp_b1.wait()
    cp_w1.wait()
    h1 = (jnp.dot(lnh16, w1_v[...], preferred_element_type=f32)
          + jnp.broadcast_to(b1_v[...].astype(f32).reshape(1, _F), (16, _F)))
    sp = jnp.log1p(jnp.exp(-jnp.abs(h1))) + jnp.maximum(h1, 0.0)
    act = (h1 * jnp.tanh(sp)).astype(bf16)
    y = jnp.zeros((16, _M), f32)
    for k, (off, n) in enumerate(_W2_PIECES):
        cp_w2(k).wait()
        y = y + jnp.dot(act[:, off:off + n], w2_v[pl.ds(off, n), :], preferred_element_type=f32)
    out_ref[...] = (h + jnp.concatenate([y[0:1, :], y[8:9, :]], axis=0)).astype(out_ref.dtype)


@jax.jit
def pallas_sequential_preLN__compressed_kv_cla__dense_activation_mish__decode_kernel(
    A_x: jax.Array,
    A_c_kv: jax.Array,
    A_w_q: jax.Array,
    A_w_uk: jax.Array,
    A_w_uv: jax.Array,
    A_w_o: jax.Array,
    B_x: jax.Array,
    B_w1: jax.Array,
    B_b1: jax.Array,
    B_w2: jax.Array,
):
    del B_x
    bf16 = jnp.bfloat16
    x2d = A_x.reshape(_B, _M)
    ckv2 = A_c_kv.reshape(_B * _SK, _DC)
    wq2 = A_w_q.reshape(_M * _H, _D)
    wuk2 = A_w_uk.reshape(_DC * _H, _D)
    wuv2 = A_w_uv.reshape(_DC * _H, _D)
    wo2 = A_w_o.reshape(_H * _D, _M)

    any_spec = pl.BlockSpec(memory_space=pl.ANY)
    out = pl.pallas_call(
        _kernel,
        out_shape=jax.ShapeDtypeStruct((_B, _M), A_x.dtype),
        in_specs=[any_spec] * 9,
        out_specs=pl.BlockSpec(memory_space=pltpu.VMEM),
        scratch_shapes=[
            pltpu.VMEM((_B, _M), bf16),
            pltpu.VMEM((_B * _SK, _DC), bf16),
            pltpu.VMEM((_M * _H, _D), bf16),
            pltpu.VMEM((_DC * _H, _D), bf16),
            pltpu.VMEM((_DC * _H, _D), bf16),
            pltpu.VMEM((_H * _D, _M), bf16),
            pltpu.VMEM((_M, _F), bf16),
            pltpu.VMEM((_F,), bf16),
            pltpu.VMEM((_F, _M), bf16),
            pltpu.VMEM((128, 1024), bf16),
            pltpu.VMEM((_B * _H, _DC), jnp.float32),
            pltpu.VMEM((_B * _H, _DC), bf16),
            pltpu.VMEM((_B, _H, 1), jnp.float32),
            pltpu.VMEM((_B, _H, 1), jnp.float32),
            pltpu.VMEM((_B, _H, _DC), jnp.float32),
            pltpu.SemaphoreType.DMA((_NSEM,)),
        ],
        compiler_params=pltpu.CompilerParams(vmem_limit_bytes=64 * 1024 * 1024),
    )(x2d, ckv2, wq2, wuk2, wuv2, wo2, B_w1, B_b1, B_w2)
    return out.reshape(_B, 1, _M)
```
